```python
import os as _os
_os.environ.setdefault("JAX_PLATFORMS", "cpu")
import jax
import jax.numpy as jnp

def _softmax(x, axis=-1):
    return jax.nn.softmax(x, axis=axis)
def _gelu(x):
    return jax.nn.gelu(x, approximate=True)
def _silu(x):
    return jax.nn.silu(x)
def _sigmoid(x):
    return jax.nn.sigmoid(x)
def _layernorm(x, axis=-1, eps=1e-5):
    m = jnp.mean(x, axis=axis, keepdims=True)
    v = jnp.var(x, axis=axis, keepdims=True)
    return (x - m) / jnp.sqrt(v + eps)
def _scatter_add(tgt, idx, src, axis=0):
    return tgt.at[idx].add(src)
def _segment_sum(src, seg, n):
    return jax.ops.segment_sum(src, seg, n)
class _Rng:
    def __init__(self, key):
        self._k = key
    def _next(self):
        self._k, sub = jax.random.split(self._k)
        return sub
    def normal(self, shape):
        return jax.random.normal(self._next(), shape, dtype=jnp.bfloat16)
    def randint(self, lo, hi, shape):
        return jax.random.randint(self._next(), shape, lo, hi, dtype=jnp.int32)
    def uniform(self, shape, lo=0.0, hi=1.0):
        return jax.random.uniform(self._next(), shape, jnp.bfloat16, lo, hi)
    def permutation(self, n):
        return jax.random.permutation(self._next(), n)


kernel_name = 'interleave_layers__mha_block__mixer_s_mlp__prompt'

def setup_inputs():
    _rng = _Rng(jax.random.key(int.from_bytes(__import__("os").urandom(4), "little")))
    _w = (lambda a: (lambda t: t.astype(jnp.bfloat16) if jnp.issubdtype(t.dtype, jnp.floating) else t)(jnp.asarray(a)))
    def _A_setup():
        B, S, D, H = 1, 2048, 448, 16
        return {
            "x": _w((lambda *s: _rng.normal(s) * 0.05)(B, S, D)),
            "wqkv": _w((lambda *s: _rng.normal(s) * 0.05)(D, 3 * D)),
            "wo": _w((lambda *s: _rng.normal(s) * 0.05)(D, D)),
        }
    _A_in = _A_setup()

    def _B_setup():
        B, S, D, F = 1, 2048, 448, 1792
        return {
            "x":  _w((lambda *s: _rng.normal(s) * 0.05)(B, S, D)),
            "w1": _w((lambda *s: _rng.normal(s) * 0.8)(D, D) * (D ** -0.5)),
            "w2": _w((lambda *s: _rng.normal(s) * 0.8)(D, D) * (D ** -0.5)),
            "w3": _w((lambda *s: _rng.normal(s) * 0.8)(D, F) * (D ** -0.5)),
            "w4": _w((lambda *s: _rng.normal(s) * 0.8)(F, D) * (F ** -0.5)),
        }
    _B_in = _B_setup()

    return {
        "A_x": _A_in["x"],
        "A_wqkv": _A_in["wqkv"],
        "A_wo": _A_in["wo"],
        "B_x": _B_in["x"],
        "B_w1": _B_in["w1"],
        "B_w2": _B_in["w2"],
        "B_w3": _B_in["w3"],
        "B_w4": _B_in["w4"],
    }

def reference(A_x, A_wqkv, A_wo, B_x, B_w1, B_w2, B_w3, B_w4):
    def _A_ref(x, wqkv, wo):
        B, S, D = x.shape
        H = 16
        Dh = D // H
        qkv = (lambda x, *d: x.transpose(*d))((x @ wqkv).reshape(B, S, 3, H, Dh), 2, 0, 3, 1, 4)
        q, k, v = qkv[0], qkv[1], qkv[2]
        scores = jnp.einsum("bhqd,bhkd->bhqk", q, k) * (Dh ** -0.5)
        p = _softmax(scores, axis=-1)
        o = jnp.einsum("bhqk,bhkd->bhqd", p, v)
        return (lambda x, *d: x.transpose(*d))(o, 0, 2, 1, 3).reshape(B, S, D) @ wo

    def _B_ref(x, w1, w2, w3, w4):
        B, S, D = x.shape
        h = _gelu(_layernorm(x, axis=-1) @ w1)
        c = D // 4
        g0 = jnp.pad(h[:, :, 0*c:1*c], ((0, 0), (1, 0), (0, 0)))[:, :S, :]
        g1 = jnp.pad(h[:, :, 1*c:2*c], ((0, 0), (0, 1), (0, 0)))[:, 1:, :]
        g2 = jnp.pad(h[:, :, 2*c:3*c], ((0, 0), (2, 0), (0, 0)))[:, :S, :]
        g3 = jnp.pad(h[:, :, 3*c:   ], ((0, 0), (0, 2), (0, 0)))[:, 2:, :]
        hs = jnp.concatenate([g0, g1, g2, g3], axis=-1) @ w2
        x1 = x + hs
        h2 = _gelu(_layernorm(x1, axis=-1) @ w3) @ w4
        return x1 + h2

    x = A_x
    x = x + _A_ref(_layernorm(x, axis=-1), A_wqkv, A_wo)
    x = x + _B_ref(_layernorm(x, axis=-1), B_w1, B_w2, B_w3, B_w4)
    x = x + _A_ref(_layernorm(x, axis=-1), A_wqkv, A_wo)
    x = x + _B_ref(_layernorm(x, axis=-1), B_w1, B_w2, B_w3, B_w4)
    return x
```

```python
import functools
import math

import jax
import jax.numpy as jnp
from jax import lax
import jax.experimental.pallas as pl
import jax.experimental.pallas.tpu as pltpu

F32 = jnp.float32
BF16 = jnp.bfloat16
U32 = jnp.uint32

S = 2048
D = 448
H = 16
DH = D // H
FF = 1792
TB = 512
NB = S // TB
HG = 4
G = H // HG
GW = HG * DH
KC = 128
NKC = S // KC
SHIFTS = (1, -1, 2, -2)
K4_LONG, K4_SHORT = 512, 384
EPS = 1e-5
Q_SCALE = (DH ** -0.5) * math.log2(math.e)
_C1 = math.sqrt(2.0 / math.pi)
BETA = (_C1 * 0.044715) ** (1.0 / 3.0)
GELU_A = _C1 / BETA
GELU_OUT = 0.5 / BETA

QKV_ROWS, QKV_ORDER = (32, 32, 48), ((3, 6, 1, 0, 4, 2, 5), (3, 1, 6, 0, 4, 2, 5))
MIX_ROWS, MIX_ORDER = (48, 48, 48, 32, 48), ((3, 1, 6, 0, 4, 2, 5),)
W3_ROWS, W3_ORDER = 32, ((3, 1, 6, 0, 4, 2, 5), (5, 1, 3, 0, 2, 4, 6))
W4_ROWS, W4_ORDER = (64, 48), ((3, 6, 1, 0, 4, 2, 5), (3, 1, 6, 0, 4, 2, 5))
QK_LEAD = 2


def _dot(a, b):
    return jnp.dot(a, b, preferred_element_type=F32)


def _pack2(lo, hi):
    return pltpu.pack_elementwise([lo, hi], packed_dtype=BF16)


def _unpack2(w):
    return [pltpu.unpack_elementwise(w, index=i, packed_dtype=BF16, unpacked_dtype=F32) for i in range(2)]


def _pack(x):
    rows, cols = x.shape
    x = x.reshape(rows // 16, 2, 8, cols)
    return _pack2(x[:, 0].reshape(rows // 2, cols), x[:, 1].reshape(rows // 2, cols))


def _pack_in_order(x):
    return pltpu.bitcast(x.astype(BF16), U32)


def _as_bf16(w):
    return pltpu.bitcast(w, BF16)


def _aligned(i, n):
    return i if isinstance(i, int) else pl.multiple_of(i, n)


def _pad128(n):
    return -(-n // 128) * 128


def _gelu_scaled(u):
    return u + u * jnp.tanh(u * (GELU_A + u * u))


class _Schedule:
    def __init__(self):
        self.zero = None
        self.pending, self.done, self.ticks, self.total = [], 0, 0, 1

    def mark(self, tile):
        bits = pltpu.bitcast(tile[0:8, 0:128], U32)
        self.zero = jnp.where((bits | 1) == 0, bits, jnp.uint32(0))

    def after(self, x):
        if self.zero is None:
            return x
        zero = jnp.concatenate([self.zero] * (x.shape[1] // 128), axis=1)
        zero = jnp.concatenate([zero] * (x.shape[0] // 8), axis=0)
        return pltpu.bitcast(pltpu.bitcast(x, U32) | zero, x.dtype)

    def tick(self):
        self.ticks += 1
        while self.done < len(self.pending) and self.done * self.total < self.ticks * len(self.pending):
            self.done += 1
            self.pending[self.done - 1]()

    def run(self, main, *sides, span=0.9):
        self.pending, self.done, self.ticks = _flat(sides), 0, 0
        self.total = max(1, int(sum(getattr(step, "ticks", 1) for step in main) * span))
        for step in main:
            step()
            if not hasattr(step, "ticks"):
                self.tick()
        assert self.done == len(self.pending)
        self.pending = []

    def loop(self, count, body):
        def wrapped(i, carry):
            self.zero = None
            body(i)
            return carry

        lax.fori_loop(0, count, wrapped, 0)
        self.zero = None


def _flat(lists):
    return [item for items in lists for item in items]


def _weave(a, b):
    order = [((i + 0.5) / len(a), 0, step) for i, step in enumerate(a)]
    order += [((i + 0.5) / len(b), 1, step) for i, step in enumerate(b)]
    return [step for _, _, step in sorted(order, key=lambda t: t[:2])]


def _split(steps, *fractions):
    cuts = [0] + [int(len(steps) * f) for f in fractions] + [len(steps)]
    return [steps[a:b] for a, b in zip(cuts, cuts[1:])]


def _colmax8(s):
    return jnp.max(s.reshape(s.shape[0] // 8, 8, s.shape[1]), axis=0)


def _quadrants(g):
    n = len(g) // 2
    return [[row[c:c + n] for row in g[r:r + n]] for r in (0, n) for c in (0, n)]


def _add(a, b):
    return [[x if y is None else y if x is None else x + y for x, y in zip(ra, rb)]
            for ra, rb in zip(a, b)]


def _sub(a, b):
    return [[x if y is None else -y if x is None else x - y for x, y in zip(ra, rb)]
            for ra, rb in zip(a, b)]


def _lhs_terms(g):
    if len(g) == 1:
        return [g[0][0]]
    a11, a12, a21, a22 = _quadrants(g)
    terms = (_add(a11, a22), _add(a21, a22), a11, a22, _add(a11, a12), _sub(a21, a11), _sub(a12, a22))
    return [t for h in terms for t in _lhs_terms(h)]


def _rhs_terms(g):
    if len(g) == 1:
        return [g[0][0]]
    b11, b12, b21, b22 = _quadrants(g)
    terms = (_add(b11, b22), b11, _sub(b12, b22), _sub(b21, b11), b22, _add(b11, b12), _add(b21, b22))
    return [t for h in terms for t in _rhs_terms(h)]


def _products(product, orders, base=0):
    if not orders:
        return [[product(base)]]
    order = orders[0]
    m = {p: _products(product, orders[1:], base * 7 + p) for p in order}

    def chain(*terms):
        terms = sorted(terms, key=lambda t: order.index(t[0]))
        if terms[0][1] < 0:
            terms[0], terms[1] = terms[1], terms[0]
        acc = m[terms[0][0]]
        for p, sign in terms[1:]:
            acc = _add(acc, m[p]) if sign > 0 else _sub(acc, m[p])
        return acc

    c11 = chain((0, 1), (3, 1), (4, -1), (6, 1))
    c12 = chain((2, 1), (4, 1))
    c21 = chain((1, 1), (3, 1))
    c22 = chain((0, 1), (1, -1), (2, 1), (5, 1))
    return [ra + rb for ra, rb in zip(c11, c12)] + [ra + rb for ra, rb in zip(c21, c22)]


def _strassen_rows(sched, a_ref, b_ref, orders, r0, rows, width=None):
    kp = a_ref.shape[2]

    def product(p):
        k = width(p) if width else kp
        b = _as_bf16(b_ref[p, :min(k // 2, b_ref.shape[1]), :])
        if b.shape[0] < k:
            b = jnp.concatenate([b, jnp.zeros((k - b.shape[0], b.shape[1]), BF16)], axis=0)
        out = _dot(_as_bf16(a_ref[p, r0 // 2:(r0 + rows) // 2, :k]), b)
        sched.mark(out)
        sched.tick()
        return out

    return [jnp.concatenate(row, axis=1) for row in _products(product, orders)]


def _rhs_steps(b_ref, rows_of, level):
    n = 2 ** level
    ks, ts = D // n, TB // n
    cache = {}

    def load(r0, k):
        part = rows_of(k * ks + r0, 16)
        cache[k] = [part[:, j * ts:(j + 1) * ts] for j in range(n)]

    def store(r0, outer):
        b11, b12, b21, b22 = _quadrants([cache[k] for k in range(n)])
        term = (lambda: _add(b11, b22), lambda: b11, lambda: _sub(b12, b22), lambda: _sub(b21, b11),
                lambda: b22, lambda: _add(b11, b12), lambda: _add(b21, b22))[outer]()
        for p, t in enumerate(_rhs_terms(term)):
            b_ref[outer * 7 ** (level - 1) + p, r0 // 2:r0 // 2 + 8, :] = _pack(t)

    def fetch_and_store(r0, outer):
        def quadrant(q):
            parts = [rows_of((2 * (q // 2) + k) * ks + r0, 16, slice(2 * ts * (q % 2), 2 * ts * (q % 2 + 1)))
                     for k in range(2)]
            return [[part[:, :ts], part[:, ts:]] for part in parts]

        first, op, second = ((0, _add, 3), (0, None, 0), (1, _sub, 3), (2, _sub, 0),
                             (3, None, 0), (0, _add, 1), (2, _add, 3))[outer]
        term = op(quadrant(first), quadrant(second)) if op else quadrant(first)
        for p, t in enumerate(_rhs_terms(term)):
            b_ref[outer * 7 + p, r0 // 2:r0 // 2 + 8, :] = _pack(t)

    steps = []
    for r0 in range(0, ks, 16):
        if level == 2:
            steps += [functools.partial(fetch_and_store, r0, outer) for outer in range(7)]
            continue
        steps += [functools.partial(load, r0, k) for k in range(n)]
        steps += [functools.partial(store, r0, outer) for outer in range(7)]
    return steps


def _tall(v, rows):
    return v if rows == 8 else jnp.concatenate([v] * (rows // 8), axis=0)


def _layernorm_steps(sched, x_ref, piece):
    stats = {}

    def accumulate(name, r0):
        tiles = [x_ref[r:r + 8, :] for r in range(r0, r0 + piece, 8)]
        if name == "var":
            mean = sched.after(stats["mean"])
            tiles = [jnp.square(x - mean) for x in tiles]
        else:
            tiles[0] = sched.after(tiles[0])
        while len(tiles) > 1:
            tiles = [a + b for a, b in zip(tiles[::2], tiles[1::2])] + tiles[len(tiles) // 2 * 2:]
        stats["acc"] = tiles[0] + stats["acc"] if r0 else tiles[0]
        if r0 + piece == D:
            total = jnp.sum(stats["acc"], axis=0, keepdims=True)
            stats[name] = jnp.broadcast_to(total * (1.0 / D), (8, TB))

    def centered(r0, rows, lanes=slice(0, TB)):
        return x_ref[r0:r0 + rows, lanes] - _tall(sched.after(stats["mean"][:, lanes]), rows)

    steps = [functools.partial(accumulate, name, r) for name in ("mean", "var") for r in range(0, D, piece)]
    return steps, centered, stats


def _normalized_rhs_steps(sched, b_ref, x_ref, level, scale, piece):
    steps, centered, stats = _layernorm_steps(sched, x_ref, piece)

    def finish():
        r = lax.rsqrt(stats["var"] + EPS)
        stats["rstd"] = r if scale is None else r * scale

    def rows_of(r0, rows, lanes=slice(0, TB)):
        return centered(r0, rows, lanes) * _tall(stats["rstd"][:, lanes], rows)

    return steps + [finish] + _rhs_steps(b_ref, rows_of, level)


def _lhs_slab_steps(sched, a_ref, block, level, word0, scale=1.0, width=None):
    def halves(i0, k0, size, lanes):
        words = [[block(i0 + i, k0 + k, lanes) for k in range(size)] for i in range(size)]
        words[0][0] = sched.after(words[0][0])
        pairs = [[(None, None) if word is None else _unpack2(word) for word in row] for row in words]
        return [[[pair[j] for pair in row] for row in pairs] for j in range(2)]

    def store(p0, lanes, even, odd):
        for p, (lo, hi) in enumerate(zip(_lhs_terms(even), _lhs_terms(odd))):
            if width and lanes.start >= width(p0 + p):
                continue
            if scale != 1.0:
                lo, hi = lo * scale, hi * scale
            a_ref[p0 + p, pl.ds(word0, 8), lanes] = _pack2(lo, hi)

    def all_terms(lanes):
        store(0, lanes, *halves(0, 0, 2 ** level, lanes))

    def outer_term(outer, lanes):
        first, op, second = ((0, _add, 3), (2, _add, 3), (0, None, 0), (3, None, 0),
                             (0, _add, 1), (2, _sub, 0), (1, _sub, 3))[outer]
        term = halves(2 * (first // 2), 2 * (first % 2), 2, lanes)
        if op:
            other = halves(2 * (second // 2), 2 * (second % 2), 2, lanes)
            term = [op(a, b) for a, b in zip(term, other)]
        store(7 * outer, lanes, *term)

    tiles = [slice(c0, c0 + 128) for c0 in range(0, a_ref.shape[2], 128)]
    if level == 2:
        return [functools.partial(outer_term, outer, lanes) for lanes in tiles for outer in range(7)]
    return [functools.partial(all_terms, lanes) for lanes in tiles]


def _transposed(sched, w, even_rows_first=False):
    w = _pack(w)
    if w.shape[1] == 128:
        w = jnp.concatenate([sched.after(w[:8]), w[8:]], axis=0)
    w = _as_bf16(w)
    if w.shape[0] % 128:
        w = jnp.concatenate([w, jnp.zeros((-w.shape[0] % 128, w.shape[1]), BF16)], axis=0)
    w = pltpu.bitcast(w.T, U32)
    if even_rows_first:
        even, odd = (half.reshape(-1, 1, 8, w.shape[1]) for half in _unpack2(w))
        w = _pack_in_order(jnp.concatenate([even, odd], axis=1).reshape(-1, w.shape[1]))
    return w


def _transpose_weight(sched, t_ref, part, parts, m_dim, columns):
    kp = t_ref.shape[1] // parts
    for col in columns:
        c0, c1 = col * 128, min(col * 128 + 128, m_dim)
        for k in range(parts):
            t_ref[c0 // 2:c1 // 2, k * kp:(k + 1) * kp] = _transposed(sched, part(k, slice(c0, c1)))


def _combine_steps(sched, a_ref, t_ref, level, first_row, j, scale=1.0):
    kp = a_ref.shape[2]

    def block(g, i, k, lanes):
        word = _aligned(first_row(i, g) // 2 + 8 * j, 8)
        return t_ref[pl.ds(word, 8), k * kp + lanes.start:k * kp + lanes.stop]

    return _flat(_lhs_slab_steps(sched, a_ref, functools.partial(block, g), level,
                                 _aligned(g * GW // 2 + 8 * j, 8), scale)
                 for g in range(a_ref.shape[1] // (GW // 2)))


def _w4_width(p):
    return K4_SHORT if p % 7 in (3, 4, 6) else K4_LONG


def _dense_steps(sched, a_ref, b_ref, orders, row_blocks, emit, width=None):
    part = 2 * a_ref.shape[1]

    def step(r0, rows):
        for i, tile in enumerate(_strassen_rows(sched, a_ref, b_ref, orders, r0, rows, width)):
            emit(i * part + r0, rows, tile)
        sched.mark(tile)

    steps, r0 = [], 0
    while r0 < part:
        for rows in row_blocks:
            steps.append(functools.partial(step, r0, rows))
            steps[-1].ticks = 7 ** len(orders)
            r0 += rows
    assert r0 == part
    return steps


def _lhs_shape(m_dim, k_dim, level):
    n = 2 ** level
    return pltpu.VMEM((7 ** level, m_dim // n // 2, _pad128(k_dim // n)), U32)


def _kernel(x_hbm, wqkv_hbm, wo_hbm, w1_hbm, w2_hbm, w3_hbm, w4_hbm, out_hbm,
            x_io, wqkv_in, wo_in, w1_in, w2_in, w3_in, w4_in,
            t_qkv, t_d, t_w3, a_qkv, a_o, a_1, a_2, a_3, a_4,
            x_t, y_t, q_t, k_s, v_t, s_a, s_b, m_s, acc_s, o_s, h_t, b_n, b_o, b_1, b_2, b_4,
            x_sem, q_sem, w_sem, o_sem):
    x_copies = [
        pltpu.make_async_copy(x_hbm.at[:, pl.ds(c * TB, TB)], x_io.at[c], x_sem.at[c])
        for c in range(NB)
    ]
    qkv_copy = pltpu.make_async_copy(wqkv_hbm, wqkv_in, q_sem)
    w_copies = [
        pltpu.make_async_copy(src, dst, w_sem.at[i])
        for i, (src, dst) in enumerate((
            (wo_hbm, wo_in), (w1_hbm, w1_in), (w2_hbm, w2_in), (w3_hbm, w3_in), (w4_hbm, w4_in)))
    ]

    def out_copy(c):
        return pltpu.make_async_copy(
            x_io.at[c], out_hbm.at[:, pl.ds(_aligned(c * TB, TB), TB)], o_sem.at[c])

    sched = _Schedule()
    run, loop = sched.run, sched.loop
    scores = (s_a, s_b)
    row32 = lax.broadcasted_iota(jnp.int32, (32, TB), 0)
    row56 = lax.broadcasted_iota(jnp.int32, (GW // 2, TB), 0)


    def qkv_steps(c, slot):
        pending = {}

        def emit(r0, rows, tile):
            index = r0 // GW
            pending.setdefault(index, []).append(tile)
            if (r0 + rows) % GW:
                return
            val = jnp.concatenate(pending.pop(index), axis=0)
            g, kind = divmod(index, 3)
            if kind == 2:
                q_t[c, g] = _pack_in_order(val * Q_SCALE)
            elif kind == 0:
                k = jnp.concatenate([val.astype(BF16), jnp.zeros((128 - GW, TB), BF16)], axis=0)
                k_s[g, c] = pltpu.bitcast(k.T, U32)
            else:
                for j in range(HG):
                    w0 = (j * DH) // 8 * 8
                    window = val[w0:w0 + 32]
                    if j * DH > w0:
                        window = pltpu.roll(window, 32 - (j * DH - w0), 0)
                    v_t[g * HG + j, c] = _pack_in_order(jnp.where(row32 < DH, window, 1.0))

        return _dense_steps(sched, a_qkv, b_n.at[slot], QKV_ORDER, QKV_ROWS, emit)

    def qkv_blocks(layer, i):
        @pl.when((layer == 0) & (i == 1))
        def _():
            x_copies[NB - 1].wait()

        for slot in range(2):
            c = 2 * i + slot
            ahead = jnp.minimum(c + 1, NB - 1)

            def widen(ahead, r0):
                x_t[ahead, r0:r0 + 64, :] = x_io[ahead, r0:r0 + 64, :].astype(F32)

            run(qkv_steps(c, slot),
                 [functools.partial(widen, ahead, r0) for r0 in range(0, D, 64)],
                 _normalized_rhs_steps(sched, b_n.at[1 - slot], x_t.at[ahead], 2, None, 32), span=0.95)


    deferred = []

    def qk_steps(c, head, slot):
        local = {}

        def step(kc):
            kb, k0, r0 = kc // (TB // KC), (kc % (TB // KC)) * KC, kc * KC
            if kc == 0:
                lo = (head % HG) * (DH // 2)
                q = jnp.where((row56 >= lo) & (row56 < lo + DH // 2), q_t[c, head // HG], jnp.uint32(0))
                local["q"] = jnp.concatenate([_as_bf16(q), jnp.zeros((128 - GW, TB), BF16)], axis=0)
            s = _dot(_as_bf16(k_s[head // HG, kb, k0 // 2:(k0 + KC) // 2, :]), local["q"])
            scores[slot][r0:r0 + KC, :] = s
            local["max"] = _colmax8(s) if kc == 0 else jnp.maximum(local["max"], _colmax8(s))
            sched.mark(s)
            if deferred:
                deferred.pop(0)()
            if kc == NKC - 1:
                m_s[slot] = jnp.broadcast_to(jnp.max(local["max"], axis=0, keepdims=True), (8, TB))

        return [functools.partial(step, kc) for kc in range(NKC)]

    def wo_rhs_steps(c, pair):
        scale = {}

        def invert(odd):
            scale[odd] = sched.after(jnp.broadcast_to(1.0 / o_s[c, odd, DH:DH + 1, :], (8, TB)))

        def store(r0, t0):
            tiles = [[o_s[c, odd, r0:r0 + 16, t:t + 128] * _tall(sched.after(scale[odd][:, t:t + 128]), 16)
                      for t in (t0, TB // 2 + t0)] for odd in range(2)]
            words = pl.ds(_aligned(pair * 16 + r0 // 2, 8), 8)
            for p, term in enumerate(_rhs_terms(tiles)):
                b_o[c, p, words, t0:t0 + 128] = _pack(term)

        return ([functools.partial(invert, odd) for odd in range(2)]
                + [functools.partial(store, r0, t0) for r0 in (0, 16) for t0 in (0, 128)])

    def pv_steps(c, pair, odd, slot, first=0, last=NKC):
        local = {}

        def step(kc):
            kb, k0, r0 = kc // (TB // KC), (kc % (TB // KC)) * KC, kc * KC
            p = jnp.exp2(scores[slot][r0:r0 + KC, :] - _tall(m_s[slot], KC)).astype(BF16)
            acc = _dot(_as_bf16(v_t[2 * pair + odd, kb, :, k0:k0 + KC]), p)
            if kc > 0:
                acc = acc + (acc_s[...] if kc == first else local["acc"])
            local["acc"] = acc
            if kc < last - 1:
                return
            if last < NKC:
                acc_s[...] = acc
                return
            o_s[c, odd] = acc
            if odd:
                deferred.extend(wo_rhs_steps(c, pair))

        return [functools.partial(step, kc) for kc in range(first, last)]

    late = NKC - QK_LEAD

    def leftover_pv_steps(pair):
        return pv_steps(NB - 2, pair, 1, 0, first=late), pv_steps(NB - 1, pair, 1, 1)

    def w4_weight_steps(j):
        def w4_block(i, k, lanes):
            if k % 2 and lanes.start >= K4_SHORT:
                return None
            rows = pl.ds(pl.multiple_of(i * GW + j * 16, 16), 16)
            c0 = (k // 2) * (FF // 2) + (k % 2) * K4_LONG
            return pltpu.bitcast(w4_in[rows, c0 + lanes.start:c0 + lanes.stop], U32)

        return _lhs_slab_steps(sched, a_4, w4_block, 2, pl.multiple_of(j * 8, 8), width=_w4_width)

    def w3_transpose_steps(j):
        def transpose(half, k):
            col = half * (FF // 256) + j
            w = w3_in[k * GW:(k + 1) * GW, pl.ds(_aligned(col * 128, 128), 128)].astype(F32)
            t_w3[pl.ds(_aligned(col * 64, 64), 64), k * 128:(k + 1) * 128] = _transposed(sched, w, even_rows_first=True)

        return [functools.partial(transpose, half, k) for half in range(2) for k in range(4)]

    def w3_weight_steps(j):
        first = [jnp.where(j < 6, 64 * j, K4_SHORT), jnp.where(j < 6, K4_LONG + 64 * j, K4_SHORT + 64)]

        def block(slab, i, k, lanes):
            word = (i // 2) * (FF // 4) + first[i % 2] // 2 + slab * 8
            return t_w3[pl.ds(pl.multiple_of(word, 8), 8), k * 128:(k + 1) * 128]

        return _flat(_lhs_slab_steps(sched, a_3, functools.partial(block, slab), 2,
                                     pl.multiple_of(j * 32 + slab * 8, 8)) for slab in range(4))

    def mixing_weight_steps(j):
        return _flat(_combine_steps(sched, a_ref, t_d.at[i], 1, lambda part, g: (2 * part + g) * GW, j, scale)
                     for i, (a_ref, scale) in enumerate(((a_o, 1.0), (a_1, 1.0), (a_2, GELU_OUT))))

    def attention_pair(pair):
        older, old = leftover_pv_steps(jnp.maximum(pair - 1, 0))
        qk, pv = [], older + old
        for unit in range(2 * NB):
            odd, c = divmod(unit, NB)
            qk += qk_steps(c, 2 * pair + odd, unit % 2)
            if unit < 2 * NB - 1:
                pv += pv_steps(c, pair, odd, unit % 2, last=NKC if unit < 2 * NB - 2 else late)
        part = jnp.minimum(pair, 6)
        run(_flat(zip(qk, pv)), mixing_weight_steps(part), w4_weight_steps(part),
            w3_weight_steps(part), span=0.75)
        assert not deferred


    def wo_steps(c):
        def emit(r0, rows, tile):
            x_t[c, r0:r0 + rows, :] += tile
        return _dense_steps(sched, a_o, b_o.at[c], MIX_ORDER, MIX_ROWS, emit)

    def w1_rhs_steps(c):
        steps, centered, stats = _layernorm_steps(sched, x_t.at[c], 8)

        def finish():
            r = lax.rsqrt(stats["var"] + EPS)
            stats["y"] = r
            stats["z"] = r * lax.rsqrt(stats["var"] * r * r + EPS) * BETA

        def rows_of(r0, rows):
            d = centered(r0, rows)
            y_t[c, r0:r0 + rows, :] = d * _tall(stats["y"], rows)
            return d * _tall(stats["z"], rows)

        return steps + [finish] + _rhs_steps(b_1.at[c], rows_of, 1)

    def w1_steps(c):
        def emit(r0, rows, tile):
            h = _gelu_scaled(tile)
            for r in range(r0, r0 + rows, 16):
                h_t[c + 1, r:r + 16, :] = pltpu.roll(h[r - r0:r - r0 + 16], SHIFTS[r // GW] % TB, 1)
        return _dense_steps(sched, a_1, b_1.at[c], MIX_ORDER, MIX_ROWS, emit)

    def w2_rhs_steps(c):
        def rows_of(r0, rows):
            shift, sl = SHIFTS[r0 // GW], slice(r0, r0 + rows)
            lane = lax.broadcasted_iota(jnp.int32, (rows, 128), 1)
            if shift > 0:
                edge = jnp.where(lane < shift, h_t[c, sl, :128], h_t[c + 1, sl, :128])
                return jnp.concatenate([sched.after(edge), h_t[c + 1, sl, 128:]], axis=1)
            edge = jnp.where(lane >= 128 + shift, h_t[c + 2, sl, TB - 128:], h_t[c + 1, sl, TB - 128:])
            return jnp.concatenate([h_t[c + 1, sl, :TB - 128], sched.after(edge)], axis=1)

        return _rhs_steps(b_2.at[c], rows_of, 1)

    def w2_steps(c):
        def emit(r0, rows, tile):
            y_t[c, r0:r0 + rows, :] += tile
        return _dense_steps(sched, a_2, b_2.at[c], MIX_ORDER, MIX_ROWS, emit)

    def token_mixing():
        def take_deferred():
            steps = deferred[:]
            deferred.clear()
            return steps

        pv = _flat(leftover_pv_steps(H // 2 - 1))
        norm2 = _split(w1_rhs_steps(2), 0.5)
        norm3 = _split(w1_rhs_steps(3), 0.05, 0.1)
        mlp0 = _split(_normalized_rhs_steps(sched, b_n.at[0], y_t.at[0], 2, BETA, 8), 0.2, 0.4, 0.65)
        run(_weave(wo_steps(0), pv[:8]))
        run(_weave(wo_steps(1), pv[8:]), take_deferred())
        run(wo_steps(2), take_deferred(), w1_rhs_steps(0))
        run(wo_steps(3), w1_rhs_steps(1))
        run(w1_steps(0), norm2[0])
        run(w1_steps(1), norm2[1], norm3[0])
        run(w1_steps(2), w2_rhs_steps(0), norm3[1])
        run(w2_steps(0), norm3[2])
        run(w1_steps(3), w2_rhs_steps(1), mlp0[0])
        run(w2_steps(1), w2_rhs_steps(2), mlp0[1])
        run(w2_steps(2), w2_rhs_steps(3), mlp0[2])
        run(w2_steps(3), mlp0[3])


    def mlp_block(layer, c):
        for r0 in range(0, FF // 4, W3_ROWS):
            g = [_gelu_scaled(u) for u in _strassen_rows(sched, a_3, b_n.at[0], W3_ORDER, r0, W3_ROWS)]
            if r0 < K4_SHORT:
                pieces = [(r0, g)]
            else:
                pieces = [(r0, [g[0], None, g[2], None]), (r0 + 64, [g[1], None, g[3], None])]
            for k0, parts in pieces:
                grid = [[None if part is None else part[:, t * 128:(t + 1) * 128] for t in range(4)]
                        for part in parts]
                for p, term in enumerate(_rhs_terms(grid)):
                    if k0 < _w4_width(p):
                        b_4[p, k0 // 2:k0 // 2 + 16, :] = _pack(term)

        def emit(r0, rows, tile):
            sl = slice(r0, r0 + rows)
            x = x_t[c, sl, :] + (y_t[c, sl, :] + tile * GELU_OUT)
            x_t[c, sl, :] = x
            x_io[c, sl, :] = x.astype(BF16)

        more = c + 1 < NB
        ahead = y_t.at[jnp.where(more, c + 1, 0)]
        run(_dense_steps(sched, a_4, b_4, W4_ORDER, W4_ROWS, emit, _w4_width),
             _normalized_rhs_steps(sched, b_n.at[0], ahead, 2, jnp.where(more, BETA, 1.0), 16), span=1.0)

        @pl.when(layer == 1)
        def _():
            out_copy(c).start()

        @pl.when(layer + c == 0)
        def _():
            y_t[0] = x_t[0]


    x_copies[0].start()
    qkv_copy.start()

    h_t[0, :, :128] = jnp.zeros((D, 128), F32)
    h_t[NB + 1, :, TB - 128:] = jnp.zeros((D, 128), F32)

    def clear_scores(kc):
        s_b[pl.ds(pl.multiple_of(kc * KC, KC), KC), :] = jnp.zeros((KC, TB), F32)

    loop(NKC, clear_scores)
    s_a[late * KC:, :] = jnp.zeros((QK_LEAD * KC, TB), F32)
    m_s[...] = jnp.zeros(m_s.shape, F32)
    acc_s[...] = jnp.zeros(acc_s.shape, F32)
    for c in (NB - 2, NB - 1):
        o_s[c, 0] = jnp.ones((32, TB), F32)

    def rows_of_weight(w_ref, parts):
        return lambda k, cols: w_ref[k * D // parts:(k + 1) * D // parts, cols].astype(F32)

    x_copies[0].wait()
    x_t[0] = x_io[0].astype(F32)
    run(_normalized_rhs_steps(sched, b_n.at[0], x_t.at[0], 2, None, 16))
    qkv_copy.wait()
    x_copies[1].start()
    x_copies[2].start()
    _transpose_weight(sched, t_qkv, rows_of_weight(wqkv_in, 4), 4, 3 * D, range(pl.cdiv(3 * D, 128)))
    for j in range(7):
        run(_combine_steps(sched, a_qkv, t_qkv, 2, lambda i, g: ((g + 1) % 3) * D + i * GW, j))
    x_copies[1].wait()
    x_copies[2].wait()
    x_copies[3].start()
    for cp in w_copies:
        cp.start()

    def wo_part(k, cols):
        w = wo_in[:, cols].astype(F32)
        pad = jnp.zeros((32 - DH, w.shape[1]), F32)
        return jnp.concatenate(
            _flat((w[head * DH:(head + 1) * DH], pad) for head in range(k, H, 2)), axis=0)

    def layer_body(layer):
        loop(NB // 2, functools.partial(qkv_blocks, layer))

        @pl.when(layer == 0)
        def _():
            for cp in w_copies:
                cp.wait()
            for i, part in enumerate((wo_part, rows_of_weight(w1_in, 2), rows_of_weight(w2_in, 2))):
                _transpose_weight(sched, t_d.at[i], part, 2, D, range(pl.cdiv(D, 128)))

            run(_flat(w3_transpose_steps(j) for j in range(7)))

        loop(H // 2, attention_pair)
        token_mixing()
        loop(NB, functools.partial(mlp_block, layer))

    loop(2, layer_body)
    for c in range(NB):
        out_copy(c).wait()


@jax.jit
def pallas_interleave_layers__mha_block__mixer_s_mlp__prompt_kernel(
    A_x: jax.Array,
    A_wqkv: jax.Array,
    A_wo: jax.Array,
    B_x: jax.Array,
    B_w1: jax.Array,
    B_w2: jax.Array,
    B_w3: jax.Array,
    B_w4: jax.Array,
):
    del B_x
    hbm = pl.BlockSpec(memory_space=pltpu.HBM)

    out = pl.pallas_call(
        _kernel,
        out_shape=jax.ShapeDtypeStruct((D, S), BF16),
        in_specs=[hbm] * 7,
        out_specs=hbm,
        scratch_shapes=[
            pltpu.VMEM((NB, D, TB), BF16),
            pltpu.VMEM((D, 3 * D), BF16),
            pltpu.VMEM((D, D), BF16),
            pltpu.VMEM((D, D), BF16),
            pltpu.VMEM((D, D), BF16),
            pltpu.VMEM((D, FF), BF16),
            pltpu.VMEM((D, FF), BF16),
            pltpu.VMEM((3 * D // 2, 512), U32),
            pltpu.VMEM((3, D // 2, 512), U32),
            pltpu.VMEM((FF // 2, 512), U32),
            _lhs_shape(3 * D, D, 2), _lhs_shape(D, D, 1), _lhs_shape(D, D, 1),
            _lhs_shape(D, D, 1), _lhs_shape(FF, D, 2), pltpu.VMEM((49, GW // 2, K4_LONG), U32),
            pltpu.VMEM((NB, D, TB), F32),
            pltpu.VMEM((NB, D, TB), F32),
            pltpu.VMEM((NB, G, GW // 2, TB), U32),
            pltpu.VMEM((G, NB, TB // 2, 128), U32),
            pltpu.VMEM((H, NB, 16, TB), U32),
            pltpu.VMEM((S, TB), F32),
            pltpu.VMEM((S, TB), F32),
            pltpu.VMEM((2, 8, TB), F32),
            pltpu.VMEM((32, TB), F32),
            pltpu.VMEM((NB, 2, 32, TB), F32),
            pltpu.VMEM((NB + 2, D, TB), F32),
            pltpu.VMEM((2, 49, D // 8, TB // 4), U32),
            pltpu.VMEM((NB, 7, 128, TB // 2), U32),
            pltpu.VMEM((NB, 7, D // 4, TB // 2), U32),
            pltpu.VMEM((NB, 7, D // 4, TB // 2), U32),
            pltpu.VMEM((49, K4_LONG // 2, TB // 4), U32),
            pltpu.SemaphoreType.DMA((NB,)),
            pltpu.SemaphoreType.DMA,
            pltpu.SemaphoreType.DMA((5,)),
            pltpu.SemaphoreType.DMA((NB,)),
        ],
        compiler_params=pltpu.CompilerParams(vmem_limit_bytes=100 * 1024 * 1024),
    )(A_x.reshape(S, D).T, A_wqkv, A_wo, B_w1, B_w2, B_w3, B_w4.T)
    return out.T.reshape(A_x.shape)
```
